```python
import jax
import jax.numpy as jnp

def _softmax(x, axis=-1):
    return jax.nn.softmax(x, axis=axis)
def _gelu(x):
    return jax.nn.gelu(x, approximate=True)
def _silu(x):
    return jax.nn.silu(x)
def _sigmoid(x):
    return jax.nn.sigmoid(x)
def _layernorm(x, axis=-1, eps=1e-5):
    m = jnp.mean(x, axis=axis, keepdims=True)
    v = jnp.var(x, axis=axis, keepdims=True)
    return (x - m) / jnp.sqrt(v + eps)
def _scatter_add(tgt, idx, src, axis=0):
    return tgt.at[idx].add(src)
def _segment_sum(src, seg, n):
    return jax.ops.segment_sum(src, seg, n)
class _Rng:
    def __init__(self, key):
        self._k = key
    def _next(self):
        self._k, sub = jax.random.split(self._k)
        return sub
    def normal(self, shape):
        return jax.random.normal(self._next(), shape, dtype=jnp.bfloat16)
    def randint(self, lo, hi, shape):
        return jax.random.randint(self._next(), shape, lo, hi, dtype=jnp.int32)
    def uniform(self, shape, lo=0.0, hi=1.0):
        return jax.random.uniform(self._next(), shape, jnp.bfloat16, lo, hi)
    def permutation(self, n):
        return jax.random.permutation(self._next(), n)


kernel_name = 'gated_mix__sliding_block_cached__glu_gated_swiglu__decode'

def setup_inputs():
    _rng = _Rng(jax.random.key(int.from_bytes(__import__("os").urandom(4), "little")))
    _w = (lambda a: (lambda t: t.astype(jnp.bfloat16) if jnp.issubdtype(t.dtype, jnp.floating) else t)(jnp.asarray(a)))
    def _A_setup():
        B, Sq, D = 1, 1, 640
        Hq, Hkv, Sk, Dh = 32, 32, 32768, 192
        assert Hq % Hkv == 0, (Hq, Hkv)
        return {
            "x": _w((lambda *s: _rng.normal(s) * 0.05)(B, Sq, D)),
            "k_cache": _w((lambda *s: _rng.normal(s) * 0.05)(B, Hkv, Sk, Dh)),
            "v_cache": _w((lambda *s: _rng.normal(s) * 0.05)(B, Hkv, Sk, Dh)),
            "wq": _w((lambda *s: _rng.normal(s) * 0.05)(D, Hq * Dh) * (D ** -0.5)),
            "wo": _w((lambda *s: _rng.normal(s) * 0.05)(Hq * Dh, D) * ((Hq * Dh) ** -0.5)),
        }
    _A_in = _A_setup()

    def _B_setup():
        B, S, D, F = 1, 1, 640, 1536
        return {
            "x": _w((lambda *s: _rng.normal(s) * 0.05)(B, S, D)),
            "w1": _w((lambda *s: _rng.normal(s) * 0.05)(D, F) * (2.0 / D) ** 0.5),
            "w3": _w((lambda *s: _rng.normal(s) * 0.05)(D, F) * (2.0 / D) ** 0.5),
            "w2": _w((lambda *s: _rng.normal(s) * 0.05)(F, D) * (2.0 / F) ** 0.5),
        }
    _B_in = _B_setup()

    return {
        "A_x": _A_in["x"],
        "A_k_cache": _A_in["k_cache"],
        "A_v_cache": _A_in["v_cache"],
        "A_wq": _A_in["wq"],
        "A_wo": _A_in["wo"],
        "B_x": _B_in["x"],
        "B_w1": _B_in["w1"],
        "B_w3": _B_in["w3"],
        "B_w2": _B_in["w2"],
        "gate_w": _w((lambda *s: _rng.normal(s) * 0.05)(640)),
    }

def reference(A_x, A_k_cache, A_v_cache, A_wq, A_wo, B_x, B_w1, B_w3, B_w2, gate_w):
    def _A_ref(x, k_cache, v_cache, wq, wo):
        B, Sq, D = x.shape
        Hq, Dh = 32, 192
        Hkv, Sk = k_cache.shape[1], k_cache.shape[2]
        W = min(4096, max(256, Sk // 4))
        rep = Hq // Hkv
        q = (lambda x, *d: x.transpose(*d))((x @ wq).reshape(B, Sq, Hq, Dh), 0, 2, 1, 3)
        k = jnp.repeat(k_cache[:, :, Sk - W:, :], rep, axis=1)
        v = jnp.repeat(v_cache[:, :, Sk - W:, :], rep, axis=1)
        scores = jnp.einsum("bhqd,bhkd->bhqk", q, k) * (Dh ** -0.5)
        p = _softmax(scores, axis=-1)
        o = jnp.einsum("bhqk,bhkd->bhqd", p, v)
        return (lambda x, *d: x.transpose(*d))(o, 0, 2, 1, 3).reshape(B, Sq, Hq * Dh) @ wo

    def _B_ref(x, w1, w3, w2):
        gate = jnp.einsum("bsd,df->bsf", x, w1)
        up = jnp.einsum("bsd,df->bsf", x, w3)
        h = _silu(gate) * up
        out = jnp.einsum("bsf,fd->bsd", h, w2)
        return out

    x = A_x
    g = _sigmoid((x * gate_w).sum(-1, keepdims=True))
    a = _A_ref(x, A_k_cache, A_v_cache, A_wq, A_wo)
    b = _B_ref(x, B_w1, B_w3, B_w2)
    return g * a + (1 - g) * b
```

```python
import jax
import jax.numpy as jnp
from jax import lax
import jax.experimental.pallas as pl
import jax.experimental.pallas.tpu as pltpu

_G = 8
_R = 512
_NB = 8


def _build(D, H, DH, SK, W, F, dtype):
    HD = H * DH
    G, R, NB = _G, _R, _NB
    GR = G * DH
    NG = H // G
    NC = GR // R
    NT = NG * 2 * NC
    assert H % G == 0 and GR % R == 0 and R % 128 == 0 and W % 128 == 0 and D % 128 == 0
    NWO = NB
    assert HD % NWO == 0 and (HD // NWO) % 128 == 0
    RW = HD // NWO
    scale = DH ** -0.5

    def kernel(x_hbm, gw_hbm, k_hbm, v_hbm, wq_hbm, wo_hbm, w1_hbm, w3_hbm, w2_hbm, o_ref,
               x_v, gw_v, wq_v, wo_v, w1_v, w3_v, w2_v, ring, qbd, s_acc, p_buf, linv, o_scr,
               sem_w, sem_wo, sem_r):
        def wcopy(src, dst, i):
            return pltpu.make_async_copy(src, dst, sem_w.at[i])

        cps = [wcopy(x_hbm, x_v, 0), wcopy(gw_hbm, gw_v, 1), wcopy(wq_hbm, wq_v, 2),
               wcopy(w1_hbm, w1_v, 3), wcopy(w3_hbm, w3_v, 4), wcopy(w2_hbm, w2_v, 5)]

        def wo_copy(c):
            return pltpu.make_async_copy(wo_hbm.at[pl.ds(c * RW, RW)],
                                         wo_v.at[pl.ds(c * RW, RW)], sem_wo.at[c])

        def ring_copy(src_hbm, row0, slot):
            return pltpu.make_async_copy(
                src_hbm.at[pl.ds(row0, R), pl.ds(SK - W, W)], ring.at[slot], sem_r.at[slot])

        def start_chunk(i):
            g = i // (2 * NC)
            ph = (i // NC) % 2
            j = i % NC
            row0 = g * GR + j * R
            slot = i % NB
            if isinstance(i, int):
                ring_copy(k_hbm if ph == 0 else v_hbm, row0, slot).start()
            else:
                row0 = pl.multiple_of(row0, R)

                @pl.when(ph == 0)
                def _():
                    ring_copy(k_hbm, row0, slot).start()

                @pl.when(ph == 1)
                def _():
                    ring_copy(v_hbm, row0, slot).start()

        def refill(i):
            @pl.when(i + NB < NT)
            def _():
                start_chunk(i + NB)

            for c in range(NWO):
                @pl.when(i == NT - NWO + c)
                def _():
                    wo_copy(c).start()

        def wait_chunk(slot):
            ring_copy(k_hbm, 0, slot).wait()

        for c in cps:
            c.start()
        for i in range(min(NB, NT)):
            start_chunk(i)

        cps[0].wait()
        cps[1].wait()
        x = x_v[...]
        xb = jnp.broadcast_to(x, (8, D))
        xf = x.astype(jnp.float32)
        gwf = gw_v[...].astype(jnp.float32)
        gsum = sum(xf[:, 128 * t:128 * (t + 1)] * gwf[t:t + 1, :] for t in range(D // 128))
        gate = jax.nn.sigmoid(jnp.sum(gsum, axis=-1, keepdims=True))

        cps[2].wait()
        row_id = lax.broadcasted_iota(jnp.int32, (G, GR), 0)
        col_id = lax.broadcasted_iota(jnp.int32, (G, GR), 1)
        bd_mask = (col_id >= row_id * DH) & (col_id < (row_id + 1) * DH)
        for g in range(NG):
            qg = jnp.dot(xb, wq_v[:, g * GR:(g + 1) * GR], preferred_element_type=jnp.float32)
            qg = qg[:1].astype(dtype).astype(jnp.float32)
            qg = jnp.broadcast_to(qg, (G, GR))
            qm = jnp.where(bd_mask, qg, 0.0).astype(dtype)
            for j in range(NC):
                qbd[g * NC + j] = qm[:, j * R:(j + 1) * R]

        cps[3].wait()
        cps[4].wait()
        gt = jnp.dot(xb, w1_v[...], preferred_element_type=jnp.float32)
        up = jnp.dot(xb, w3_v[...], preferred_element_type=jnp.float32)
        hh = (gt * jax.nn.sigmoid(gt) * up).astype(dtype)
        cps[5].wait()
        b = jnp.dot(hh, w2_v[...], preferred_element_type=jnp.float32)[:1]
        bmix = (1.0 - gate) * b

        def k_body(j, g):
            i = g * 2 * NC + j
            slot = i % NB
            wait_chunk(slot)
            s = jnp.dot(qbd[g * NC + j], ring[slot], preferred_element_type=jnp.float32)

            @pl.when(j == 0)
            def _():
                s_acc[...] = s

            @pl.when(j > 0)
            def _():
                s_acc[...] += s

            refill(i)
            return g

        def v_body(j, g):
            i = g * 2 * NC + NC + j
            slot = i % NB
            wait_chunk(slot)
            oc = lax.dot_general(p_buf[...], ring[slot], (((1,), (1,)), ((), ())),
                                 preferred_element_type=jnp.float32)
            oc = oc * linv[...]
            r_id = lax.broadcasted_iota(jnp.int32, (G, R), 0)
            c_id = lax.broadcasted_iota(jnp.int32, (G, R), 1) + j * R
            m = (c_id >= r_id * DH) & (c_id < (r_id + 1) * DH)
            o_scr[g * NC + j] = jnp.where(m, oc, 0.0).astype(dtype)
            refill(i)
            return g

        def group_body(g, _):
            lax.fori_loop(0, NC, k_body, g)
            s = s_acc[...] * scale
            mx = jnp.max(s, axis=-1, keepdims=True)
            e = jnp.exp(s - mx)
            l = jnp.sum(e, axis=-1, keepdims=True)
            p_buf[...] = e.astype(dtype)
            linv[...] = 1.0 / l
            lax.fori_loop(0, NC, v_body, g)
            return 0

        lax.fori_loop(0, NG, group_body, 0)

        acc = jnp.zeros((G, D), jnp.float32)
        for c in range(NWO):
            wo_copy(c).wait()
            pos = c * RW
            while pos < (c + 1) * RW:
                blk = pos // R
                lo = pos - blk * R
                hi = min(R, (c + 1) * RW - blk * R)
                acc += jnp.dot(o_scr[blk, :, lo:hi], wo_v[blk * R + lo:blk * R + hi, :],
                               preferred_element_type=jnp.float32)
                pos = blk * R + hi
        a = jnp.sum(acc, axis=0, keepdims=True)
        o_ref[...] = (gate * a + bmix).astype(o_ref.dtype)

    return pl.pallas_call(
        kernel,
        out_shape=jax.ShapeDtypeStruct((1, D), dtype),
        in_specs=[pl.BlockSpec(memory_space=pl.ANY)] * 9,
        out_specs=pl.BlockSpec(memory_space=pltpu.VMEM),
        scratch_shapes=[
            pltpu.VMEM((1, D), dtype), pltpu.VMEM((D // 128, 128), dtype),
            pltpu.VMEM((D, HD), dtype), pltpu.VMEM((HD, D), dtype),
            pltpu.VMEM((D, F), dtype), pltpu.VMEM((D, F), dtype), pltpu.VMEM((F, D), dtype),
            pltpu.VMEM((NB, R, W), dtype),
            pltpu.VMEM((HD // R, G, R), dtype),
            pltpu.VMEM((G, W), jnp.float32),
            pltpu.VMEM((G, W), dtype),
            pltpu.VMEM((G, 1), jnp.float32),
            pltpu.VMEM((HD // R, G, R), dtype),
            pltpu.SemaphoreType.DMA((6,)),
            pltpu.SemaphoreType.DMA((NWO,)),
            pltpu.SemaphoreType.DMA((NB,)),
        ],
        compiler_params=pltpu.CompilerParams(vmem_limit_bytes=100 * 1024 * 1024),
    )


@jax.jit
def pallas_gated_mix__sliding_block_cached__glu_gated_swiglu__decode_kernel(
    A_x: jax.Array,
    A_k_cache: jax.Array,
    A_v_cache: jax.Array,
    A_wq: jax.Array,
    A_wo: jax.Array,
    B_x: jax.Array,
    B_w1: jax.Array,
    B_w3: jax.Array,
    B_w2: jax.Array,
    gate_w: jax.Array,
):
    del B_x
    B, Sq, D = A_x.shape
    _, H, SK, DH = A_k_cache.shape
    assert B == 1 and Sq == 1 and A_wq.shape == (D, H * DH)
    W = min(4096, max(256, SK // 4))
    F = B_w1.shape[1]
    x2 = A_x.reshape(1, D)
    gw2 = gate_w.reshape(D // 128, 128)
    kT = A_k_cache.reshape(H, SK, DH).transpose(0, 2, 1).reshape(H * DH, SK)
    vT = A_v_cache.reshape(H, SK, DH).transpose(0, 2, 1).reshape(H * DH, SK)
    out = _build(D, H, DH, SK, W, F, A_x.dtype)(x2, gw2, kT, vT, A_wq, A_wo, B_w1, B_w3, B_w2)
    return out.reshape(B, Sq, D)
```

```python
import jax
import jax.numpy as jnp
from jax import lax
import jax.experimental.pallas as pl
import jax.experimental.pallas.tpu as pltpu

_G = 8
_R = 384
_NB = 8
_WO_SPLIT = (8, 8, 8, 8, 8, 5, 2, 1)


def _build(D, H, DH, SK, W, F, dtype):
    HD = H * DH
    G, R, NB = _G, _R, _NB
    GR = G * DH
    NG = H // G
    NC = GR // R
    NT = NG * 2 * NC
    assert H % G == 0 and GR % R == 0 and R % 128 == 0 and W % 128 == 0 and D % 128 == 0
    unit = HD // sum(_WO_SPLIT)
    assert unit * sum(_WO_SPLIT) == HD and unit % 128 == 0
    wo_rows = [unit * n for n in _WO_SPLIT]
    wo_off = [sum(wo_rows[:c]) for c in range(len(wo_rows))]
    NWO = len(wo_rows)
    assert NWO <= NT
    scale = DH ** -0.5

    def kernel(x_hbm, gw_hbm, k_hbm, v_hbm, wq_hbm, wo_hbm, w1_hbm, w3_hbm, w2_hbm, o_ref,
               x_v, gw_v, wq_v, wo_v, w1_v, w3_v, w2_v, ring, qbd, s_acc, p_buf, linv, o_scr,
               sem_w, sem_wo, sem_r):
        def wcopy(src, dst, i):
            return pltpu.make_async_copy(src, dst, sem_w.at[i])

        cps = [wcopy(x_hbm, x_v, 0), wcopy(gw_hbm, gw_v, 1), wcopy(wq_hbm, wq_v, 2),
               wcopy(w1_hbm, w1_v, 3), wcopy(w3_hbm, w3_v, 4), wcopy(w2_hbm, w2_v, 5)]

        def wo_copy(c):
            return pltpu.make_async_copy(wo_hbm.at[pl.ds(wo_off[c], wo_rows[c])],
                                         wo_v.at[pl.ds(wo_off[c], wo_rows[c])], sem_wo.at[c])

        def ring_copy(src_hbm, row0, slot):
            return pltpu.make_async_copy(
                src_hbm.at[pl.ds(row0, R), pl.ds(SK - W, W)], ring.at[slot], sem_r.at[slot])

        def start_chunk(i):
            g = i // (2 * NC)
            ph = (i // NC) % 2
            j = i % NC
            row0 = g * GR + j * R
            slot = i % NB
            if isinstance(i, int):
                ring_copy(k_hbm if ph == 0 else v_hbm, row0, slot).start()
            else:
                row0 = pl.multiple_of(row0, R)

                @pl.when(ph == 0)
                def _():
                    ring_copy(k_hbm, row0, slot).start()

                @pl.when(ph == 1)
                def _():
                    ring_copy(v_hbm, row0, slot).start()

        def refill(i):
            @pl.when(i + NB < NT)
            def _():
                start_chunk(i + NB)

            for c in range(NWO):
                @pl.when(i == NT - NWO + c)
                def _():
                    wo_copy(c).start()

        def wait_chunk(src_hbm, g, j, slot):
            ring_copy(src_hbm, pl.multiple_of(g * GR + j * R, R), slot).wait()

        for c in cps:
            c.start()
        for i in range(min(NB, NT)):
            start_chunk(i)

        cps[0].wait()
        cps[1].wait()
        x = x_v[...]
        xb = jnp.broadcast_to(x, (8, D))
        xf = x.astype(jnp.float32)
        gwf = gw_v[...].astype(jnp.float32)
        gsum = sum(xf[:, 128 * t:128 * (t + 1)] * gwf[t:t + 1, :] for t in range(D // 128))
        gate = jax.nn.sigmoid(jnp.sum(gsum, axis=-1, keepdims=True))

        cps[2].wait()
        row_id = lax.broadcasted_iota(jnp.int32, (G, GR), 0)
        col_id = lax.broadcasted_iota(jnp.int32, (G, GR), 1)
        bd_mask = (col_id >= row_id * DH) & (col_id < (row_id + 1) * DH)
        for g in range(NG):
            qg = jnp.dot(xb, wq_v[:, g * GR:(g + 1) * GR], preferred_element_type=jnp.float32)
            qg = qg[:1].astype(dtype).astype(jnp.float32)
            qg = jnp.broadcast_to(qg, (G, GR))
            qm = jnp.where(bd_mask, qg, 0.0).astype(dtype)
            for j in range(NC):
                qbd[g * NC + j] = qm[:, j * R:(j + 1) * R]

        cps[3].wait()
        cps[4].wait()
        gt = jnp.dot(xb, w1_v[...], preferred_element_type=jnp.float32)
        up = jnp.dot(xb, w3_v[...], preferred_element_type=jnp.float32)
        hh = (gt * jax.nn.sigmoid(gt) * up).astype(dtype)
        cps[5].wait()
        b = jnp.dot(hh, w2_v[...], preferred_element_type=jnp.float32)[:1]
        bmix = (1.0 - gate) * b

        def k_body(j, g):
            i = g * 2 * NC + j
            slot = i % NB
            wait_chunk(k_hbm, g, j, slot)
            s = jnp.dot(qbd[g * NC + j], ring[slot], preferred_element_type=jnp.float32)

            @pl.when(j == 0)
            def _():
                s_acc[...] = s

            @pl.when(j > 0)
            def _():
                s_acc[...] += s

            refill(i)
            return g

        def v_body(j, g):
            i = g * 2 * NC + NC + j
            slot = i % NB
            wait_chunk(v_hbm, g, j, slot)
            oc = lax.dot_general(p_buf[...], ring[slot], (((1,), (1,)), ((), ())),
                                 preferred_element_type=jnp.float32)
            oc = oc * linv[...]
            r_id = lax.broadcasted_iota(jnp.int32, (G, R), 0)
            c_id = lax.broadcasted_iota(jnp.int32, (G, R), 1) + j * R
            m = (c_id >= r_id * DH) & (c_id < (r_id + 1) * DH)
            o_scr[g * NC + j] = jnp.where(m, oc, 0.0).astype(dtype)
            refill(i)
            return g

        def group_body(g, _):
            lax.fori_loop(0, NC, k_body, g)
            s = s_acc[...] * scale
            mx = jnp.max(s, axis=-1, keepdims=True)
            e = jnp.exp(s - mx)
            l = jnp.sum(e, axis=-1, keepdims=True)
            p_buf[...] = e.astype(dtype)
            linv[...] = 1.0 / l
            lax.fori_loop(0, NC, v_body, g)
            return 0

        lax.fori_loop(0, NG, group_body, 0)

        acc = jnp.zeros((G, D), jnp.float32)
        for c in range(NWO):
            wo_copy(c).wait()
            pos, end = wo_off[c], wo_off[c] + wo_rows[c]
            while pos < end:
                blk = pos // R
                lo = pos - blk * R
                hi = min(R, end - blk * R)
                acc += jnp.dot(o_scr[blk, :, lo:hi], wo_v[blk * R + lo:blk * R + hi, :],
                               preferred_element_type=jnp.float32)
                pos = blk * R + hi
        a = jnp.sum(acc, axis=0, keepdims=True)
        o_ref[...] = (gate * a + bmix).astype(o_ref.dtype)

    return pl.pallas_call(
        kernel,
        out_shape=jax.ShapeDtypeStruct((1, D), dtype),
        in_specs=[pl.BlockSpec(memory_space=pl.ANY)] * 9,
        out_specs=pl.BlockSpec(memory_space=pltpu.VMEM),
        scratch_shapes=[
            pltpu.VMEM((1, D), dtype), pltpu.VMEM((D // 128, 128), dtype),
            pltpu.VMEM((D, HD), dtype), pltpu.VMEM((HD, D), dtype),
            pltpu.VMEM((D, F), dtype), pltpu.VMEM((D, F), dtype), pltpu.VMEM((F, D), dtype),
            pltpu.VMEM((NB, R, W), dtype),
            pltpu.VMEM((HD // R, G, R), dtype),
            pltpu.VMEM((G, W), jnp.float32),
            pltpu.VMEM((G, W), dtype),
            pltpu.VMEM((G, 1), jnp.float32),
            pltpu.VMEM((HD // R, G, R), dtype),
            pltpu.SemaphoreType.DMA((6,)),
            pltpu.SemaphoreType.DMA((NWO,)),
            pltpu.SemaphoreType.DMA((NB,)),
        ],
        compiler_params=pltpu.CompilerParams(vmem_limit_bytes=72 * 1024 * 1024,
                                             disable_semaphore_checks=True),
    )


@jax.jit
def pallas_gated_mix__sliding_block_cached__glu_gated_swiglu__decode_kernel(
    A_x: jax.Array,
    A_k_cache: jax.Array,
    A_v_cache: jax.Array,
    A_wq: jax.Array,
    A_wo: jax.Array,
    B_x: jax.Array,
    B_w1: jax.Array,
    B_w3: jax.Array,
    B_w2: jax.Array,
    gate_w: jax.Array,
):
    del B_x
    B, Sq, D = A_x.shape
    _, H, SK, DH = A_k_cache.shape
    assert B == 1 and Sq == 1 and A_wq.shape == (D, H * DH)
    W = min(4096, max(256, SK // 4))
    F = B_w1.shape[1]
    x2 = A_x.reshape(1, D)
    gw2 = gate_w.reshape(D // 128, 128)
    kT = A_k_cache.reshape(H, SK, DH).transpose(0, 2, 1).reshape(H * DH, SK)
    vT = A_v_cache.reshape(H, SK, DH).transpose(0, 2, 1).reshape(H * DH, SK)
    out = _build(D, H, DH, SK, W, F, A_x.dtype)(x2, gw2, kT, vT, A_wq, A_wo, B_w1, B_w3, B_w2)
    return out.reshape(B, Sq, D)
```

```python
import jax
import jax.numpy as jnp
from jax import lax
import jax.experimental.pallas as pl
import jax.experimental.pallas.tpu as pltpu

_G = 8
_R = 384
_NB = 8
_WO_SPLIT = (8, 8, 8, 8, 8, 4, 2, 1)
_WO_VPU = (96, 32)


def _build(D, H, DH, SK, W, F, dtype):
    HD = H * DH
    G, R, NB = _G, _R, _NB
    GR = G * DH
    NG = H // G
    NC = GR // R
    NT = NG * 2 * NC
    assert H % G == 0 and GR % R == 0 and R % 128 == 0 and W % 128 == 0 and D % 128 == 0
    RV = sum(_WO_VPU)
    wo_rows = [128 * n for n in _WO_SPLIT]
    wo_rows[0] += HD - RV - sum(wo_rows)
    NMX = len(wo_rows)
    assert RV == 128 and R % RV == 0 and HD % 128 == 0 and wo_rows[0] > 0
    wo_rows += list(_WO_VPU)
    wo_off = [sum(wo_rows[:c]) for c in range(len(wo_rows))]
    NWO = len(wo_rows)
    assert NWO <= NT
    scale = DH ** -0.5

    def kernel(x_hbm, gw_hbm, k_hbm, v_hbm, wq_hbm, wo_hbm, w1_hbm, w3_hbm, w2_hbm, o_ref,
               x_v, gw_v, wq_v, wo_v, w1_v, w3_v, w2_v, ring, qbd, s_acc, p_buf, linv, o_scr,
               sem_w, sem_wo, sem_r):
        def wcopy(src, dst, i):
            return pltpu.make_async_copy(src, dst, sem_w.at[i])

        cps = [wcopy(x_hbm, x_v, 0), wcopy(gw_hbm, gw_v, 1), wcopy(wq_hbm, wq_v, 2),
               wcopy(w1_hbm, w1_v, 3), wcopy(w3_hbm, w3_v, 4), wcopy(w2_hbm, w2_v, 5)]

        def wo_copy(c):
            return pltpu.make_async_copy(wo_hbm.at[pl.ds(wo_off[c], wo_rows[c])],
                                         wo_v.at[pl.ds(wo_off[c], wo_rows[c])], sem_wo.at[c])

        def ring_copy(src_hbm, row0, slot):
            return pltpu.make_async_copy(
                src_hbm.at[pl.ds(row0, R), pl.ds(SK - W, W)], ring.at[slot], sem_r.at[slot])

        def start_chunk(i):
            g = i // (2 * NC)
            ph = (i // NC) % 2
            j = i % NC
            row0 = g * GR + j * R
            slot = i % NB
            if isinstance(i, int):
                ring_copy(k_hbm if ph == 0 else v_hbm, row0, slot).start()
            else:
                row0 = pl.multiple_of(row0, R)

                @pl.when(ph == 0)
                def _():
                    ring_copy(k_hbm, row0, slot).start()

                @pl.when(ph == 1)
                def _():
                    ring_copy(v_hbm, row0, slot).start()

        def refill(i):
            @pl.when(i + NB < NT)
            def _():
                start_chunk(i + NB)

            for c in range(NWO):
                @pl.when(i == NT - NWO + c)
                def _():
                    wo_copy(c).start()

        def wait_chunk(src_hbm, g, j, slot):
            ring_copy(src_hbm, pl.multiple_of(g * GR + j * R, R), slot).wait()

        for c in cps:
            c.start()
        for i in range(min(NB, NT)):
            start_chunk(i)

        cps[0].wait()
        cps[1].wait()
        x = x_v[...]
        xb = jnp.broadcast_to(x, (8, D))
        xf = x.astype(jnp.float32)
        gwf = gw_v[...].astype(jnp.float32)
        gsum = sum(xf[:, 128 * t:128 * (t + 1)] * gwf[t:t + 1, :] for t in range(D // 128))
        gate = jax.nn.sigmoid(jnp.sum(gsum, axis=-1, keepdims=True))

        cps[2].wait()
        row_id = lax.broadcasted_iota(jnp.int32, (G, GR), 0)
        col_id = lax.broadcasted_iota(jnp.int32, (G, GR), 1)
        bd_mask = (col_id >= row_id * DH) & (col_id < (row_id + 1) * DH)
        for g in range(NG):
            qg = jnp.dot(xb, wq_v[:, g * GR:(g + 1) * GR], preferred_element_type=jnp.float32)
            qg = qg[:1].astype(dtype).astype(jnp.float32)
            qg = jnp.broadcast_to(qg, (G, GR))
            qm = jnp.where(bd_mask, qg, 0.0).astype(dtype)
            for j in range(NC):
                qbd[g * NC + j] = qm[:, j * R:(j + 1) * R]

        cps[3].wait()
        cps[4].wait()
        gt = jnp.dot(xb, w1_v[...], preferred_element_type=jnp.float32)
        up = jnp.dot(xb, w3_v[...], preferred_element_type=jnp.float32)
        hh = (gt * jax.nn.sigmoid(gt) * up).astype(dtype)
        cps[5].wait()
        b = jnp.dot(hh, w2_v[...], preferred_element_type=jnp.float32)[:1]
        bmix = (1.0 - gate) * b

        def k_body(j, g):
            i = g * 2 * NC + j
            slot = i % NB
            wait_chunk(k_hbm, g, j, slot)
            s = jnp.dot(qbd[g * NC + j], ring[slot], preferred_element_type=jnp.float32)

            @pl.when(j == 0)
            def _():
                s_acc[...] = s

            @pl.when(j > 0)
            def _():
                s_acc[...] += s

            refill(i)
            return g

        def v_body(j, g):
            i = g * 2 * NC + NC + j
            slot = i % NB
            wait_chunk(v_hbm, g, j, slot)
            oc = lax.dot_general(p_buf[...], ring[slot], (((1,), (1,)), ((), ())),
                                 preferred_element_type=jnp.float32)
            oc = oc * linv[...]
            r_id = lax.broadcasted_iota(jnp.int32, (G, R), 0)
            c_id = lax.broadcasted_iota(jnp.int32, (G, R), 1) + j * R
            m = (c_id >= r_id * DH) & (c_id < (r_id + 1) * DH)
            o_scr[g * NC + j] = jnp.where(m, oc, 0.0).astype(dtype)
            refill(i)
            return g

        def group_body(g, _):
            lax.fori_loop(0, NC, k_body, g)
            s = s_acc[...] * scale
            mx = jnp.max(s, axis=-1, keepdims=True)
            e = jnp.exp(s - mx)
            l = jnp.sum(e, axis=-1, keepdims=True)
            p_buf[...] = e.astype(dtype)
            linv[...] = 1.0 / l
            lax.fori_loop(0, NC, v_body, g)
            return 0

        lax.fori_loop(0, NG, group_body, 0)

        ot = o_scr[HD // R - 1, :, R - RV:R].astype(jnp.float32)
        ocol = jnp.sum(ot, axis=0, keepdims=True)
        ocol = jnp.transpose(jnp.broadcast_to(ocol, (128, RV)))

        acc = jnp.zeros((G, D), jnp.float32)
        for c in range(NMX):
            wo_copy(c).wait()
            pos, end = wo_off[c], wo_off[c] + wo_rows[c]
            while pos < end:
                blk = pos // R
                lo = pos - blk * R
                hi = min(R, end - blk * R)
                acc += jnp.dot(o_scr[blk, :, lo:hi], wo_v[blk * R + lo:blk * R + hi, :],
                               preferred_element_type=jnp.float32)
                pos = blk * R + hi
        for c in range(NMX, NWO):
            wo_copy(c).wait()
            r0, n = wo_off[c], wo_rows[c]
            wv = wo_v[r0:r0 + n, :].astype(jnp.float32)
            oc = ocol[r0 - (HD - RV):r0 - (HD - RV) + n, :]
            pr = wv * jnp.concatenate([oc] * (D // 128), axis=1)
            for t in range(n // 8):
                acc = acc + pr[8 * t:8 * t + 8]
        a = jnp.sum(acc, axis=0, keepdims=True)
        o_ref[...] = (gate * a + bmix).astype(o_ref.dtype)

    return pl.pallas_call(
        kernel,
        out_shape=jax.ShapeDtypeStruct((1, D), dtype),
        in_specs=[pl.BlockSpec(memory_space=pl.ANY)] * 9,
        out_specs=pl.BlockSpec(memory_space=pltpu.VMEM),
        scratch_shapes=[
            pltpu.VMEM((1, D), dtype), pltpu.VMEM((D // 128, 128), dtype),
            pltpu.VMEM((D, HD), dtype), pltpu.VMEM((HD, D), dtype),
            pltpu.VMEM((D, F), dtype), pltpu.VMEM((D, F), dtype), pltpu.VMEM((F, D), dtype),
            pltpu.VMEM((NB, R, W), dtype),
            pltpu.VMEM((HD // R, G, R), dtype),
            pltpu.VMEM((G, W), jnp.float32),
            pltpu.VMEM((G, W), dtype),
            pltpu.VMEM((G, 1), jnp.float32),
            pltpu.VMEM((HD // R, G, R), dtype),
            pltpu.SemaphoreType.DMA((6,)),
            pltpu.SemaphoreType.DMA((NWO,)),
            pltpu.SemaphoreType.DMA((NB,)),
        ],
        compiler_params=pltpu.CompilerParams(vmem_limit_bytes=72 * 1024 * 1024,
                                             disable_semaphore_checks=True),
    )


@jax.jit
def pallas_gated_mix__sliding_block_cached__glu_gated_swiglu__decode_kernel(
    A_x: jax.Array,
    A_k_cache: jax.Array,
    A_v_cache: jax.Array,
    A_wq: jax.Array,
    A_wo: jax.Array,
    B_x: jax.Array,
    B_w1: jax.Array,
    B_w3: jax.Array,
    B_w2: jax.Array,
    gate_w: jax.Array,
):
    del B_x
    B, Sq, D = A_x.shape
    _, H, SK, DH = A_k_cache.shape
    assert B == 1 and Sq == 1 and A_wq.shape == (D, H * DH)
    W = min(4096, max(256, SK // 4))
    F = B_w1.shape[1]
    x2 = A_x.reshape(1, D)
    gw2 = gate_w.reshape(D // 128, 128)
    kT = A_k_cache.reshape(H, SK, DH).transpose(0, 2, 1).reshape(H * DH, SK)
    vT = A_v_cache.reshape(H, SK, DH).transpose(0, 2, 1).reshape(H * DH, SK)
    out = _build(D, H, DH, SK, W, F, A_x.dtype)(x2, gw2, kT, vT, A_wq, A_wo, B_w1, B_w3, B_w2)
    return out.reshape(B, Sq, D)
```
